```python
import os as _os
_os.environ.setdefault("JAX_PLATFORMS", "cpu")
import jax
import jax.numpy as jnp

def _softmax(x, axis=-1):
    return jax.nn.softmax(x, axis=axis)
def _gelu(x):
    return jax.nn.gelu(x, approximate=True)
def _silu(x):
    return jax.nn.silu(x)
def _sigmoid(x):
    return jax.nn.sigmoid(x)
def _layernorm(x, axis=-1, eps=1e-5):
    m = jnp.mean(x, axis=axis, keepdims=True)
    v = jnp.var(x, axis=axis, keepdims=True)
    return (x - m) / jnp.sqrt(v + eps)
def _scatter_add(tgt, idx, src, axis=0):
    return tgt.at[idx].add(src)
def _segment_sum(src, seg, n):
    return jax.ops.segment_sum(src, seg, n)
class _Rng:
    def __init__(self, key):
        self._k = key
    def _next(self):
        self._k, sub = jax.random.split(self._k)
        return sub
    def normal(self, shape):
        return jax.random.normal(self._next(), shape, dtype=jnp.bfloat16)
    def randint(self, lo, hi, shape):
        return jax.random.randint(self._next(), shape, lo, hi, dtype=jnp.int32)
    def uniform(self, shape, lo=0.0, hi=1.0):
        return jax.random.uniform(self._next(), shape, jnp.bfloat16, lo, hi)
    def permutation(self, n):
        return jax.random.permutation(self._next(), n)


kernel_name = 'concat_heads__sliding_block_cached__sliding_block_cached__decode'

def setup_inputs():
    _rng = _Rng(jax.random.key(int.from_bytes(__import__("os").urandom(4), "little")))
    _w = (lambda a: (lambda t: t.astype(jnp.bfloat16) if jnp.issubdtype(t.dtype, jnp.floating) else t)(jnp.asarray(a)))
    def _A_setup():
        B, Sq, D = 4, 1, 576
        Hq, Hkv, Sk, Dh = 32, 16, 8192, 128
        assert Hq % Hkv == 0, (Hq, Hkv)
        return {
            "x": _w((lambda *s: _rng.normal(s) * 0.8)(B, Sq, D)),
            "k_cache": _w((lambda *s: _rng.normal(s) * 0.8)(B, Hkv, Sk, Dh)),
            "v_cache": _w((lambda *s: _rng.normal(s) * 0.05)(B, Hkv, Sk, Dh)),
            "wq": _w((lambda *s: _rng.normal(s) * 0.8)(D, Hq * Dh) * (D ** -0.5)),
            "wo": _w((lambda *s: _rng.normal(s) * 0.05)(Hq * Dh, D) * ((Hq * Dh) ** -0.5)),
        }
    _A_in = _A_setup()

    def _B_setup():
        B, Sq, D = 4, 1, 576
        Hq, Hkv, Sk, Dh = 32, 16, 8192, 128
        assert Hq % Hkv == 0, (Hq, Hkv)
        return {
            "x": _w((lambda *s: _rng.normal(s) * 0.8)(B, Sq, D)),
            "k_cache": _w((lambda *s: _rng.normal(s) * 0.8)(B, Hkv, Sk, Dh)),
            "v_cache": _w((lambda *s: _rng.normal(s) * 0.05)(B, Hkv, Sk, Dh)),
            "wq": _w((lambda *s: _rng.normal(s) * 0.8)(D, Hq * Dh) * (D ** -0.5)),
            "wo": _w((lambda *s: _rng.normal(s) * 0.05)(Hq * Dh, D) * ((Hq * Dh) ** -0.5)),
        }
    _B_in = _B_setup()

    return {
        "A_x": _A_in["x"],
        "A_k_cache": _A_in["k_cache"],
        "A_v_cache": _A_in["v_cache"],
        "A_wq": _A_in["wq"],
        "A_wo": _A_in["wo"],
        "B_x": _B_in["x"],
        "B_k_cache": _B_in["k_cache"],
        "B_v_cache": _B_in["v_cache"],
        "B_wq": _B_in["wq"],
        "B_wo": _B_in["wo"],
    }

def reference(A_x, A_k_cache, A_v_cache, A_wq, A_wo, B_x, B_k_cache, B_v_cache, B_wq, B_wo):
    def _A_ref(x, k_cache, v_cache, wq, wo):
        B, Sq, D = x.shape
        Hq, Dh = 32, 128
        Hkv, Sk = k_cache.shape[1], k_cache.shape[2]
        W = min(4096, max(256, Sk // 4))
        rep = Hq // Hkv
        q = (lambda x, *d: x.transpose(*d))((x @ wq).reshape(B, Sq, Hq, Dh), 0, 2, 1, 3)
        k = jnp.repeat(k_cache[:, :, Sk - W:, :], rep, axis=1)
        v = jnp.repeat(v_cache[:, :, Sk - W:, :], rep, axis=1)
        scores = jnp.einsum("bhqd,bhkd->bhqk", q, k) * (Dh ** -0.5)
        p = _softmax(scores, axis=-1)
        o = jnp.einsum("bhqk,bhkd->bhqd", p, v)
        return (lambda x, *d: x.transpose(*d))(o, 0, 2, 1, 3).reshape(B, Sq, Hq * Dh) @ wo

    def _B_ref(x, k_cache, v_cache, wq, wo):
        B, Sq, D = x.shape
        Hq, Dh = 32, 128
        Hkv, Sk = k_cache.shape[1], k_cache.shape[2]
        W = min(4096, max(256, Sk // 4))
        rep = Hq // Hkv
        q = (lambda x, *d: x.transpose(*d))((x @ wq).reshape(B, Sq, Hq, Dh), 0, 2, 1, 3)
        k = jnp.repeat(k_cache[:, :, Sk - W:, :], rep, axis=1)
        v = jnp.repeat(v_cache[:, :, Sk - W:, :], rep, axis=1)
        scores = jnp.einsum("bhqd,bhkd->bhqk", q, k) * (Dh ** -0.5)
        p = _softmax(scores, axis=-1)
        o = jnp.einsum("bhqk,bhkd->bhqd", p, v)
        return (lambda x, *d: x.transpose(*d))(o, 0, 2, 1, 3).reshape(B, Sq, Hq * Dh) @ wo

    a = _A_ref(A_x, A_k_cache, A_v_cache, A_wq, A_wo)
    b = _B_ref(B_x, B_k_cache, B_v_cache, B_wq, B_wo)
    return jnp.concatenate([a, b], axis=-1)
```

```python
import jax
import jax.numpy as jnp
from jax import lax
import jax.experimental.pallas as pl
import jax.experimental.pallas.tpu as pltpu

_HQ = 32
_DH = 128
_TS = 128
_PAT = (0, 1, 1, 1)
_NH = 2
_SKEW = 3
_LOOKAHEAD = 3


def _kv_order(nt):
    per = nt // _NH
    o = []
    for i in range(4 * nt):
        a, k = i % 4, i // 4
        o.append((a, ((k % _NH) * per + k // _NH + _SKEW * a) % nt, _PAT[i % 4]))
    return o


def _w_order(nrows):
    nch = nrows // 8 * 2
    half = nch // 2
    per = half // _NH
    o = []
    for i in range(2 * nch):
        s, k = i % 4, i // 4
        a, hi = s % 2, s // 2
        j = hi * half + ((k % _NH) * per + k // _NH + _SKEW * s) % half
        o.append((a, j // 2, j % 2, _PAT[i % 4]))
    return o


@jax.jit
def pallas_concat_heads__sliding_block_cached__sliding_block_cached__decode_kernel(
    A_x: jax.Array,
    A_k_cache: jax.Array,
    A_v_cache: jax.Array,
    A_wq: jax.Array,
    A_wo: jax.Array,
    B_x: jax.Array,
    B_k_cache: jax.Array,
    B_v_cache: jax.Array,
    B_wq: jax.Array,
    B_wo: jax.Array,
):
    B, Sq, D = A_x.shape
    _, Hkv, Sk, Dh = A_k_cache.shape
    assert Sq == 1 and B == 4 and D == 576 and Dh == _DH and _HQ == 2 * Hkv
    W = min(4096, max(256, Sk // 4))
    N = _HQ * Dh
    NC = N // 2
    NT = W // _TS
    L = _LOOKAHEAD
    R = L + 1
    scale = Dh ** -0.5
    NU = B * Hkv
    KVO = _kv_order(NT)
    WU = [(128 * c, 128) for c in range(4)] + [(512, 64)]
    FU = [(512, 0, 64)] + [(128 * c, 64 + 128 * c, 128) for c in range(4)]
    nW, nF = len(WU), len(FU)

    def kernel(ax, ak, av, awq, awo, bx, bk, bv, bwq, bwo, out_ref,
               xbuf, wqbuf, wobuf, kvbuf, qacc, qtab, otab, sem_x, sem_w, sem_k, sem_f):
        kv_arrs = (ak, av, bk, bv)
        wq_arrs = (awq, bwq)
        wo_arrs = (awo, bwo)

        def half(o, part):
            if part is None:
                return o
            return o[part * len(o) // 2:(part + 1) * len(o) // 2]

        def issue_w(c, part=None):
            r0, nr = WU[c]
            for a, s, hf, p in half(_w_order(nr), part):
                pltpu.make_async_copy(
                    wq_arrs[a].at[pl.ds(r0 + 8 * s, 8), pl.ds(hf * NC, NC)],
                    wqbuf.at[a, pl.ds(r0 + 8 * s, 8), pl.ds(hf * NC, NC)],
                    sem_w.at[c]).start(priority=p)

        def wait_w(c):
            r0, nr = WU[c]
            r = wqbuf.at[:, pl.ds(r0, nr), :]
            pltpu.make_async_copy(r, r, sem_w.at[c]).wait()

        def issue_f(c, part=None):
            ra, rb, nr = FU[c]
            for a, s, hf, p in half(_w_order(nr), part):
                r0 = (ra, rb)[a]
                pltpu.make_async_copy(
                    wo_arrs[a].at[pl.ds(r0 + 8 * s, 8), pl.ds(hf * NC, NC)],
                    wobuf.at[a, pl.ds(r0 + 8 * s, 8), pl.ds(hf * NC, NC)],
                    sem_f.at[2 * c + a]).start(priority=p)

        def wait_f(c, a):
            ra, rb, nr = FU[c]
            r = wobuf.at[a, pl.ds((ra, rb)[a], nr), :]
            pltpu.make_async_copy(r, r, sem_f.at[2 * c + a]).wait()

        def issue_k(u, part=None):
            slot = u % R
            h, b = u // B, u % B
            for a, t, p in half(KVO, part):
                pltpu.make_async_copy(
                    kv_arrs[a].at[b, h, pl.ds(Sk - W + t * _TS, _TS), :],
                    kvbuf.at[slot, a, pl.ds(t * _TS, _TS), :],
                    sem_k.at[slot]).start(priority=p)

        def wait_k(u):
            slot = u % R
            pltpu.make_async_copy(kvbuf.at[slot], kvbuf.at[slot], sem_k.at[slot]).wait()

        stream = ([("w", c) for c in range(nW)] + [("k", u) for u in range(NU)]
                  + [("f", c) for c in range(nF)])

        def issue(item, part=None):
            kind, i = item
            {"w": issue_w, "k": issue_k, "f": issue_f}[kind](i, part)

        row = lax.broadcasted_iota(jnp.int32, (8, Dh), 0)

        xcp = [pltpu.make_async_copy(x, xbuf.at[i], sem_x.at[i]) for i, x in enumerate((ax, bx))]
        for c in xcp:
            c.start()
        for i in range(L):
            issue(stream[i])
        otab[...] = jnp.zeros_like(otab)
        for c in xcp:
            c.wait()
        x8 = []
        for p in range(2):
            xv = xbuf[p].astype(jnp.float32)
            x8.append(jnp.concatenate([xv, xv], axis=0).astype(jnp.bfloat16))

        for c in range(nW):
            r0, nr = WU[c]
            wait_w(c)
            for p in range(2):
                issue(stream[c + L], p)
                part = jnp.dot(x8[p][:, r0:r0 + nr], wqbuf[p, r0:r0 + nr, :],
                               preferred_element_type=jnp.float32)
                if c == 0:
                    qacc[p] = part
                elif c < nW - 1:
                    qacc[p] += part
                else:
                    q = (qacc[p] + part).astype(jnp.bfloat16).astype(jnp.float32)
                    for h in range(Hkv):
                        qtab[p * Hkv + h] = jnp.where(
                            row < 4, q[:, (2 * h) * Dh:(2 * h + 1) * Dh],
                            q[:, (2 * h + 1) * Dh:(2 * h + 2) * Dh])

        def attn(p, u):
            slot = u % R
            h, b = u // B, u % B
            q = qtab[p * Hkv + h].astype(jnp.bfloat16)
            s = lax.dot_general(q, kvbuf[slot, 2 * p], (((1,), (1,)), ((), ())),
                                preferred_element_type=jnp.float32) * scale
            m = jnp.max(s, axis=-1, keepdims=True)
            e = jnp.exp(s - m)
            l = jnp.sum(e, axis=-1, keepdims=True)
            o = jnp.dot(e.astype(jnp.bfloat16), kvbuf[slot, 2 * p + 1],
                        preferred_element_type=jnp.float32) / l
            otab[p * Hkv + h] = jnp.where((row & 3) == b, o, otab[p * Hkv + h])

        def body(u, c):
            wait_k(u)
            for p in range(2):
                issue_k(u + L, p)
                attn(p, u)
            return c

        lax.fori_loop(0, NU - L, body, 0)
        for u in range(NU - L, NU):
            wait_k(u)
            for p in range(2):
                issue(stream[nW + u + L], p)
                attn(p, u)

        olhs = []
        for p in range(2):
            pieces = []
            for h in range(Hkv):
                o = otab[p * Hkv + h]
                pieces.append(o.astype(jnp.bfloat16))
                pieces.append(pltpu.roll(o, 4, axis=0).astype(jnp.bfloat16))
            olhs.append(jnp.concatenate(pieces, axis=1))
        for c in range(nF):
            ra, rb, nr = FU[c]
            for p in range(2):
                if c + L < nF:
                    issue(("f", c + L), p)
                wait_f(c, p)
                r0 = (ra, rb)[p]
                res = lax.dot_general(olhs[p], wobuf[p, r0:r0 + nr, :], (((1,), (1,)), ((), ())),
                                      preferred_element_type=jnp.float32)
                out_ref[:, p * D + r0:p * D + r0 + nr] = res[:B].astype(out_ref.dtype)

    hbm = pl.BlockSpec(memory_space=pltpu.HBM)
    out = pl.pallas_call(
        kernel,
        in_specs=[hbm] * 10,
        out_specs=pl.BlockSpec(memory_space=pltpu.VMEM),
        out_shape=jax.ShapeDtypeStruct((B, 2 * D), A_x.dtype),
        scratch_shapes=[
            pltpu.VMEM((2, B, D), jnp.bfloat16),
            pltpu.VMEM((2, D, N), jnp.bfloat16),
            pltpu.VMEM((2, D, N), jnp.bfloat16),
            pltpu.VMEM((R, 4, W, Dh), jnp.bfloat16),
            pltpu.VMEM((2, 8, N), jnp.float32),
            pltpu.VMEM((2 * Hkv, 8, Dh), jnp.float32),
            pltpu.VMEM((2 * Hkv, 8, Dh), jnp.float32),
            pltpu.SemaphoreType.DMA((2,)),
            pltpu.SemaphoreType.DMA((nW,)),
            pltpu.SemaphoreType.DMA((R,)),
            pltpu.SemaphoreType.DMA((2 * nF,)),
        ],
        compiler_params=pltpu.CompilerParams(
            vmem_limit_bytes=64 * 1024 * 1024, disable_bounds_checks=True),
    )(A_x.reshape(B, D), A_k_cache, A_v_cache, A_wq, A_wo.T,
      B_x.reshape(B, D), B_k_cache, B_v_cache, B_wq, B_wo.T)
    return out.reshape(B, 1, 2 * D)
```

```python
import jax
import jax.numpy as jnp
from jax import lax
import jax.experimental.pallas as pl
import jax.experimental.pallas.tpu as pltpu

_HQ = 32
_DH = 128
_TS = 128
_CC = 1024
_PAT = (0, 1, 1, 1)
_LAG = 96
_TOP = 24
_LAST = (2048, 1024, 1024)
_DELAY = 16
_NSLOT = 3


@jax.jit
def pallas_concat_heads__sliding_block_cached__sliding_block_cached__decode_kernel(
    A_x: jax.Array,
    A_k_cache: jax.Array,
    A_v_cache: jax.Array,
    A_wq: jax.Array,
    A_wo: jax.Array,
    B_x: jax.Array,
    B_k_cache: jax.Array,
    B_v_cache: jax.Array,
    B_wq: jax.Array,
    B_wo: jax.Array,
):
    B, Sq, D = A_x.shape
    _, Hkv, Sk, Dh = A_k_cache.shape
    assert Sq == 1 and B == 4 and D == 576 and Dh == _DH and _HQ == 2 * Hkv
    W = min(4096, max(256, Sk // 4))
    N = _HQ * Dh
    QR = D // 4
    NSTRIP = QR // 8
    NTILE = QR // 16
    NT = W // _TS
    NU = B * Hkv // 2
    R = _NSLOT
    LT, TT = _LAG // 8, _TOP // 8
    scale = Dh ** -0.5
    assert W % _TS == 0 and LT < NT and 3 * TT <= NT and sum(_LAST) == N

    sord = [4 * a + s for s in range(4) for a in range(2)]
    groups, copies = [], []

    def add_group(items, tile, c0, c1):
        for k, item in enumerate(items):
            copies.append(item + (_PAT[k % 4], len(groups)))
        groups.append((tile, c0, c1))

    for i in range(NTILE - 1):
        add_group([(st, j, c, _CC) for j in (2 * i, 2 * i + 1)
                   for c in range(0, N, _CC) for st in sord], i, 0, N)
    col = 0
    for w in _LAST:
        add_group([(st, j, c, _CC) for c in range(col, col + w, _CC)
                   for j in (NSTRIP - 2, NSTRIP - 1) for st in sord], NTILE - 1, col, col + w)
        col += w
    NG = len(groups)
    lo, hi = [], []
    for st, j, c, cc, p, g in copies:
        if p == 0 and g < NG - 1:
            hi.append((len(lo), (st, j, c, cc, 0, g)))
        else:
            lo.append((st, j, c, cc, 1, g))
    fcopies, k0 = [], 0
    for n1, item in enumerate(lo):
        while k0 < len(hi) and hi[k0][0] + _DELAY <= n1:
            fcopies.append(hi[k0][1])
            k0 += 1
        fcopies.append(item)
    fcopies.extend(item for _, item in hi[k0:])
    gend = [max(i for i, x in enumerate(fcopies) if x[5] == g) + 1 for g in range(NG)]

    def kernel(ax, ak, av, awq, awo, bx, bk, bv, bwq, bwo, out_ref,
               xbuf, wqbuf, wobuf, kvbuf, qtab, otab, zref, sem_x, sem_w, sem_k, sem_f):
        kv_arrs = (ak, av, bk, bv)
        wq_arrs = (awq, bwq)
        wo_arrs = (awo, bwo)

        zref[0] = 0

        def block(fn):
            def body(_, c):
                fn()
                return c
            lax.fori_loop(0, zref[0] + 1, body, 0)

        def unit_bh(u, j):
            return u % B, (u // B) * 2 + j

        def issue_k(u, t0, t1, pinned=True):
            if t1 <= t0:
                return

            def go():
                slot = u % R
                for t in range(t0, t1):
                    for j in range(2):
                        b, h = unit_bh(u, j)
                        for a in range(4):
                            pltpu.make_async_copy(
                                kv_arrs[a].at[b, h, pl.ds(Sk - W + t * _TS, _TS), :],
                                kvbuf.at[slot, j * 4 + a, pl.ds(t * _TS, _TS), :],
                                sem_k.at[slot]).start(priority=_PAT[a])
            if pinned:
                block(go)
            else:
                go()

        def issue_rel(u, t0, t1, pinned=True):
            issue_k(u, t0, min(t1, NT), pinned)
            issue_k(u + 1, max(t0, NT) - NT, t1 - NT, pinned)

        def wait_k(u):
            slot = u % R
            pltpu.make_async_copy(kvbuf.at[slot], kvbuf.at[slot], sem_k.at[slot]).wait()

        fpos = [0]

        def issue_f(upto):
            upto = min(upto, len(fcopies))
            if upto <= fpos[0]:
                return
            items = fcopies[fpos[0]:upto]
            fpos[0] = upto

            def go():
                z = zref[0]
                for st, j, c, cc, p, g in items:
                    i = j // 2
                    dst = 16 * ((st + i) % 8) + 8 * (j % 2)
                    pltpu.make_async_copy(
                        wo_arrs[st // 4].at[pl.ds(QR * (st % 4) + 8 * j, 8), pl.ds(c, cc)],
                        wobuf.at[i, pl.ds(dst, 8), pl.ds(c, cc)],
                        sem_f.at[g + z]).start(priority=p)
            block(go)

        def wait_f(g):
            i, c0, c1 = groups[g]
            r = wobuf.at[i, :, pl.ds(c0, c1 - c0)]
            pltpu.make_async_copy(r, r, sem_f.at[g]).wait()

        row = lax.broadcasted_iota(jnp.int32, (8, Dh), 0)
        lane = lax.broadcasted_iota(jnp.int32, (8, Dh), 1)

        xcp = [pltpu.make_async_copy(x, xbuf.at[i], sem_x.at[i])
               for i, x in enumerate((ax, bx))]
        for c in xcp:
            c.start()

        def issue_w(j, carry):
            for c in range(0, N, _CC):
                for k, st in enumerate(sord):
                    r0 = pl.multiple_of(QR * (st % 4) + 8 * j, 8)
                    pltpu.make_async_copy(
                        wq_arrs[st // 4].at[pl.ds(r0, 8), pl.ds(c, _CC)],
                        wqbuf.at[st // 4, pl.ds(r0, 8), pl.ds(c, _CC)],
                        sem_w.at[0]).start(priority=_PAT[k % 4])
            return carry

        lax.fori_loop(0, NSTRIP, issue_w, 0)
        otab[...] = jnp.zeros_like(otab)
        for c in xcp:
            c.wait()
        x8 = []
        for p in range(2):
            xv = xbuf[p].astype(jnp.float32)
            x8.append(jnp.concatenate([xv, xv], axis=0).astype(jnp.bfloat16))
        issue_rel(0, 0, LT, pinned=False)
        pltpu.make_async_copy(wqbuf, wqbuf, sem_w.at[0]).wait()

        for k in range(8):
            p, cq = k // 4, k % 4
            q = jnp.dot(x8[p], wqbuf[p, :, cq * 1024:(cq + 1) * 1024],
                        preferred_element_type=jnp.float32)
            q = q.astype(jnp.bfloat16).astype(jnp.float32)
            for hh in range(4):
                qtab[p * Hkv + cq * 4 + hh] = jnp.where(
                    row < 4, q[:, (2 * hh) * Dh:(2 * hh + 1) * Dh],
                    q[:, (2 * hh + 1) * Dh:(2 * hh + 2) * Dh])
            issue_rel(0, LT + NT * k // 8, LT + NT * (k + 1) // 8)

        def attn(p, j, u):
            slot = u % R
            b, h = unit_bh(u, j)
            q = qtab[p * Hkv + h].astype(jnp.bfloat16)
            s = lax.dot_general(q, kvbuf[slot, j * 4 + 2 * p], (((1,), (1,)), ((), ())),
                                preferred_element_type=jnp.float32) * scale
            m = jnp.max(s, axis=-1, keepdims=True)
            e = jnp.exp(s - m)
            l = jnp.sum(e, axis=-1, keepdims=True)
            o = jnp.dot(e.astype(jnp.bfloat16), kvbuf[slot, j * 4 + 2 * p + 1],
                        preferred_element_type=jnp.float32) / l
            otab[p * Hkv + h] = jnp.where((row & 3) == b, o, otab[p * Hkv + h])

        cuts = [LT, LT + TT, LT + 2 * TT, LT + 3 * TT, LT + NT]

        def kv_step(u, carry):
            wait_k(u)
            for k in range(4):
                attn(k // 2, k % 2, u)
                issue_rel(u + 1, cuts[k], cuts[k + 1], pinned=False)
            return carry

        lax.fori_loop(0, NU - 2, kv_step, 0)
        wait_k(NU - 2)
        for k in range(4):
            attn(k // 2, k % 2, NU - 2)
            issue_k(NU - 1, cuts[k], min(cuts[k + 1], NT))
            issue_f((cuts[k + 1] - NT) * 8)
        wait_k(NU - 1)
        for k in range(4):
            attn(k // 2, k % 2, NU - 1)
            issue_f(fpos[0] + _TOP)

        pieces = []
        for h in range(Hkv):
            oa, ob = otab[h], otab[Hkv + h]
            pieces.append(jnp.where(row < 4, oa, pltpu.roll(ob, 4, axis=0)).astype(jnp.bfloat16))
            pieces.append(jnp.where(row < 4, pltpu.roll(oa, 4, axis=0), ob).astype(jnp.bfloat16))
        olhs = jnp.concatenate(pieces, axis=1)
        acc = None
        for g in range(NG):
            i, c0, c1 = groups[g]
            issue_f(max(gend[g] + _LAG, fpos[0] + _TOP))
            wait_f(g)
            res = lax.dot_general(olhs[:, c0:c1], wobuf[i, :, c0:c1], (((1,), (1,)), ((), ())),
                                  preferred_element_type=jnp.float32)
            if c0 > 0:
                res = res + acc
            if c1 < N:
                acc = res
            else:
                is_b = (((lane >> 4) + (8 - i % 8)) & 7) >= 4
                res = jnp.where(is_b, pltpu.roll(res, 4, axis=0), res)
                res = res[:B].astype(out_ref.dtype)
                for st in range(8):
                    l0 = 16 * ((st + i) % 8)
                    oc = QR * st + 16 * i
                    out_ref[:, oc:oc + 16] = res[:, l0:l0 + 16]

    hbm = pl.BlockSpec(memory_space=pltpu.HBM)
    out = pl.pallas_call(
        kernel,
        in_specs=[hbm] * 10,
        out_specs=pl.BlockSpec(memory_space=pltpu.VMEM),
        out_shape=jax.ShapeDtypeStruct((B, 2 * D), A_x.dtype),
        scratch_shapes=[
            pltpu.VMEM((2, B, D), jnp.bfloat16),
            pltpu.VMEM((2, D, N), jnp.bfloat16),
            pltpu.VMEM((NTILE, 128, N), jnp.bfloat16),
            pltpu.VMEM((R, 8, W, Dh), jnp.bfloat16),
            pltpu.VMEM((2 * Hkv, 8, Dh), jnp.float32),
            pltpu.VMEM((2 * Hkv, 8, Dh), jnp.float32),
            pltpu.SMEM((1,), jnp.int32),
            pltpu.SemaphoreType.DMA((2,)),
            pltpu.SemaphoreType.DMA((1,)),
            pltpu.SemaphoreType.DMA((R,)),
            pltpu.SemaphoreType.DMA((NG,)),
        ],
        compiler_params=pltpu.CompilerParams(
            vmem_limit_bytes=48 * 1024 * 1024,
            disable_bounds_checks=True,
            disable_semaphore_checks=True),
    )(A_x.reshape(B, D), A_k_cache, A_v_cache, A_wq, A_wo.T,
      B_x.reshape(B, D), B_k_cache, B_v_cache, B_wq, B_wo.T)
    return out.reshape(B, 1, 2 * D)
```

```python
import jax
import jax.numpy as jnp
from jax import lax
import jax.experimental.pallas as pl
import jax.experimental.pallas.tpu as pltpu

_HQ = 32
_DH = 128
_TS = 128
_CC = 1024
_PAT = (0, 1, 1, 1)
_LAG = 96
_TOP = 24
_LAST = (2048, 1024, 1024)
_DELAY = 16
_NSLOT = 3
_SHIFT = (0, 0, 16, 16)


@jax.jit
def pallas_concat_heads__sliding_block_cached__sliding_block_cached__decode_kernel(
    A_x: jax.Array,
    A_k_cache: jax.Array,
    A_v_cache: jax.Array,
    A_wq: jax.Array,
    A_wo: jax.Array,
    B_x: jax.Array,
    B_k_cache: jax.Array,
    B_v_cache: jax.Array,
    B_wq: jax.Array,
    B_wo: jax.Array,
):
    B, Sq, D = A_x.shape
    _, Hkv, Sk, Dh = A_k_cache.shape
    assert Sq == 1 and B == 4 and D == 576 and Dh == _DH and _HQ == 2 * Hkv
    W = min(4096, max(256, Sk // 4))
    N = _HQ * Dh
    QR = D // 4
    NSTRIP = QR // 8
    NTILE = QR // 16
    NT = W // _TS
    NU = B * Hkv // 2
    R = _NSLOT
    LT, TT = _LAG // 8, _TOP // 8
    scale = Dh ** -0.5
    assert W % _TS == 0 and LT < NT and 3 * TT <= NT and sum(_LAST) == N

    def kv_rows(a, t):
        sh = _SHIFT[a]
        lo, hi = t * _TS + sh, (t + 1) * _TS + sh
        rows = [(max(lo, 0), min(hi, W) - max(lo, 0))]
        if t == 0 and lo > 0:
            rows.insert(0, (0, lo))
        if t == NT - 1 and hi < W:
            rows.append((hi, W - hi))
        return rows

    sord = [4 * a + s for s in range(4) for a in range(2)]
    groups, copies = [], []

    def add_group(items, tile, c0, c1):
        for k, item in enumerate(items):
            copies.append(item + (_PAT[k % 4], len(groups)))
        groups.append((tile, c0, c1))

    for i in range(NTILE - 1):
        add_group([(st, j, c, _CC) for j in (2 * i, 2 * i + 1)
                   for c in range(0, N, _CC) for st in sord], i, 0, N)
    col = 0
    for w in _LAST:
        add_group([(st, j, c, _CC) for c in range(col, col + w, _CC)
                   for j in (NSTRIP - 2, NSTRIP - 1) for st in sord], NTILE - 1, col, col + w)
        col += w
    NG = len(groups)
    lo, hi = [], []
    for st, j, c, cc, p, g in copies:
        if p == 0 and g < NG - 1:
            hi.append((len(lo), (st, j, c, cc, 0, g)))
        else:
            lo.append((st, j, c, cc, 1, g))
    fcopies, k0 = [], 0
    for n1, item in enumerate(lo):
        while k0 < len(hi) and hi[k0][0] + _DELAY <= n1:
            fcopies.append(hi[k0][1])
            k0 += 1
        fcopies.append(item)
    fcopies.extend(item for _, item in hi[k0:])
    gend = [max(i for i, x in enumerate(fcopies) if x[5] == g) + 1 for g in range(NG)]

    def kernel(ax, ak, av, awq, awo, bx, bk, bv, bwq, bwo, out_ref,
               xbuf, wqbuf, wobuf, kvbuf, qtab, otab, zref, sem_x, sem_w, sem_k, sem_f):
        kv_arrs = (ak, av, bk, bv)
        wq_arrs = (awq, bwq)
        wo_arrs = (awo, bwo)

        zref[0] = 0

        def block(fn):
            def body(_, c):
                fn()
                return c
            lax.fori_loop(0, zref[0] + 1, body, 0)

        def unit_bh(u, j):
            return u % B, (u // B) * 2 + j

        def issue_k(u, t0, t1, pinned=True):
            if t1 <= t0:
                return

            def go():
                slot = u % R
                for t in range(t0, t1):
                    for j in range(2):
                        b, h = unit_bh(u, j)
                        for a in range(4):
                            for r0, nr in kv_rows(a, t):
                                pltpu.make_async_copy(
                                    kv_arrs[a].at[b, h, pl.ds(Sk - W + r0, nr), :],
                                    kvbuf.at[slot, j * 4 + a, pl.ds(r0, nr), :],
                                    sem_k.at[slot]).start(priority=_PAT[a])
            if pinned:
                block(go)
            else:
                go()

        def issue_rel(u, t0, t1, pinned=True):
            issue_k(u, t0, min(t1, NT), pinned)
            issue_k(u + 1, max(t0, NT) - NT, t1 - NT, pinned)

        def wait_k(u):
            slot = u % R
            pltpu.make_async_copy(kvbuf.at[slot], kvbuf.at[slot], sem_k.at[slot]).wait()

        fpos = [0]

        def issue_f(upto):
            upto = min(upto, len(fcopies))
            if upto <= fpos[0]:
                return
            items = fcopies[fpos[0]:upto]
            fpos[0] = upto

            def go():
                z = zref[0]
                for st, j, c, cc, p, g in items:
                    i = j // 2
                    dst = 16 * ((st + i) % 8) + 8 * (j % 2)
                    pltpu.make_async_copy(
                        wo_arrs[st // 4].at[pl.ds(QR * (st % 4) + 8 * j, 8), pl.ds(c, cc)],
                        wobuf.at[i, pl.ds(dst, 8), pl.ds(c, cc)],
                        sem_f.at[g + z]).start(priority=p)
            block(go)

        def wait_f(g):
            i, c0, c1 = groups[g]
            r = wobuf.at[i, :, pl.ds(c0, c1 - c0)]
            pltpu.make_async_copy(r, r, sem_f.at[g]).wait()

        row = lax.broadcasted_iota(jnp.int32, (8, Dh), 0)
        lane = lax.broadcasted_iota(jnp.int32, (8, Dh), 1)

        xcp = [pltpu.make_async_copy(x, xbuf.at[i], sem_x.at[i])
               for i, x in enumerate((ax, bx))]
        for c in xcp:
            c.start()

        def issue_w(j, carry):
            for c in range(0, N, _CC):
                for k, st in enumerate(sord):
                    r0 = pl.multiple_of(QR * (st % 4) + 8 * j, 8)
                    pltpu.make_async_copy(
                        wq_arrs[st // 4].at[pl.ds(r0, 8), pl.ds(c, _CC)],
                        wqbuf.at[st // 4, pl.ds(r0, 8), pl.ds(c, _CC)],
                        sem_w.at[0]).start(priority=_PAT[k % 4])
            return carry

        lax.fori_loop(0, NSTRIP, issue_w, 0)
        otab[...] = jnp.zeros_like(otab)
        for c in xcp:
            c.wait()
        x8 = []
        for p in range(2):
            xv = xbuf[p].astype(jnp.float32)
            x8.append(jnp.concatenate([xv, xv], axis=0).astype(jnp.bfloat16))
        issue_rel(0, 0, LT, pinned=False)
        pltpu.make_async_copy(wqbuf, wqbuf, sem_w.at[0]).wait()

        for k in range(8):
            p, cq = k // 4, k % 4
            q = jnp.dot(x8[p], wqbuf[p, :, cq * 1024:(cq + 1) * 1024],
                        preferred_element_type=jnp.float32)
            q = q.astype(jnp.bfloat16).astype(jnp.float32)
            for hh in range(4):
                qtab[p * Hkv + cq * 4 + hh] = jnp.where(
                    row < 4, q[:, (2 * hh) * Dh:(2 * hh + 1) * Dh],
                    q[:, (2 * hh + 1) * Dh:(2 * hh + 2) * Dh])
            issue_rel(0, LT + NT * k // 8, LT + NT * (k + 1) // 8)

        def attn(p, j, u):
            slot = u % R
            b, h = unit_bh(u, j)
            q = qtab[p * Hkv + h].astype(jnp.bfloat16)
            s = lax.dot_general(q, kvbuf[slot, j * 4 + 2 * p], (((1,), (1,)), ((), ())),
                                preferred_element_type=jnp.float32) * scale
            m = jnp.max(s, axis=-1, keepdims=True)
            e = jnp.exp(s - m)
            l = jnp.sum(e, axis=-1, keepdims=True)
            o = jnp.dot(e.astype(jnp.bfloat16), kvbuf[slot, j * 4 + 2 * p + 1],
                        preferred_element_type=jnp.float32) / l
            otab[p * Hkv + h] = jnp.where((row & 3) == b, o, otab[p * Hkv + h])

        cuts = [LT, LT + TT, LT + 2 * TT, LT + 3 * TT, LT + NT]

        def kv_step(u, carry):
            wait_k(u)
            for k in range(4):
                attn(k // 2, k % 2, u)
                issue_rel(u + 1, cuts[k], cuts[k + 1], pinned=False)
            return carry

        lax.fori_loop(0, NU - 2, kv_step, 0)
        wait_k(NU - 2)
        for k in range(4):
            attn(k // 2, k % 2, NU - 2)
            issue_k(NU - 1, cuts[k], min(cuts[k + 1], NT))
            issue_f((cuts[k + 1] - NT) * 8)
        wait_k(NU - 1)
        for k in range(4):
            attn(k // 2, k % 2, NU - 1)
            issue_f(fpos[0] + _TOP)

        pieces = []
        for h in range(Hkv):
            oa, ob = otab[h], otab[Hkv + h]
            pieces.append(jnp.where(row < 4, oa, pltpu.roll(ob, 4, axis=0)).astype(jnp.bfloat16))
            pieces.append(jnp.where(row < 4, pltpu.roll(oa, 4, axis=0), ob).astype(jnp.bfloat16))
        olhs = jnp.concatenate(pieces, axis=1)
        acc = None
        for g in range(NG):
            i, c0, c1 = groups[g]
            issue_f(max(gend[g] + _LAG, fpos[0] + _TOP))
            wait_f(g)
            res = lax.dot_general(olhs[:, c0:c1], wobuf[i, :, c0:c1], (((1,), (1,)), ((), ())),
                                  preferred_element_type=jnp.float32)
            if c0 > 0:
                res = res + acc
            if c1 < N:
                acc = res
            else:
                is_b = (((lane >> 4) + (8 - i % 8)) & 7) >= 4
                res = jnp.where(is_b, pltpu.roll(res, 4, axis=0), res)
                res = res[:B].astype(out_ref.dtype)
                for st in range(8):
                    l0 = 16 * ((st + i) % 8)
                    oc = QR * st + 16 * i
                    out_ref[:, oc:oc + 16] = res[:, l0:l0 + 16]

    hbm = pl.BlockSpec(memory_space=pltpu.HBM)
    out = pl.pallas_call(
        kernel,
        in_specs=[hbm] * 10,
        out_specs=pl.BlockSpec(memory_space=pltpu.VMEM),
        out_shape=jax.ShapeDtypeStruct((B, 2 * D), A_x.dtype),
        scratch_shapes=[
            pltpu.VMEM((2, B, D), jnp.bfloat16),
            pltpu.VMEM((2, D, N), jnp.bfloat16),
            pltpu.VMEM((NTILE, 128, N), jnp.bfloat16),
            pltpu.VMEM((R, 8, W, Dh), jnp.bfloat16),
            pltpu.VMEM((2 * Hkv, 8, Dh), jnp.float32),
            pltpu.VMEM((2 * Hkv, 8, Dh), jnp.float32),
            pltpu.SMEM((1,), jnp.int32),
            pltpu.SemaphoreType.DMA((2,)),
            pltpu.SemaphoreType.DMA((1,)),
            pltpu.SemaphoreType.DMA((R,)),
            pltpu.SemaphoreType.DMA((NG,)),
        ],
        compiler_params=pltpu.CompilerParams(
            vmem_limit_bytes=48 * 1024 * 1024,
            disable_bounds_checks=True,
            disable_semaphore_checks=True),
    )(A_x.reshape(B, D), A_k_cache, A_v_cache, A_wq, A_wo.T,
      B_x.reshape(B, D), B_k_cache, B_v_cache, B_wq, B_wo.T)
    return out.reshape(B, 1, 2 * D)
```

```python
import jax
import jax.numpy as jnp
from jax import lax
import jax.experimental.pallas as pl
import jax.experimental.pallas.tpu as pltpu

_HQ = 32
_DH = 128
_TS = 128
_CC = 1024
_PAT = (0, 1, 1, 1)
_KPAT = (1, 0, 1, 1)
_LAG = 96
_TOP = 24
_LAST = (2048, 1024, 1024)
_DELAY = 16
_NSLOT = 3
_SHIFT = (0, 0, 16, 16)


@jax.jit
def pallas_concat_heads__sliding_block_cached__sliding_block_cached__decode_kernel(
    A_x: jax.Array,
    A_k_cache: jax.Array,
    A_v_cache: jax.Array,
    A_wq: jax.Array,
    A_wo: jax.Array,
    B_x: jax.Array,
    B_k_cache: jax.Array,
    B_v_cache: jax.Array,
    B_wq: jax.Array,
    B_wo: jax.Array,
):
    B, Sq, D = A_x.shape
    _, Hkv, Sk, Dh = A_k_cache.shape
    assert Sq == 1 and B == 4 and D == 576 and Dh == _DH and _HQ == 2 * Hkv
    W = min(4096, max(256, Sk // 4))
    N = _HQ * Dh
    QR = D // 4
    NSTRIP = QR // 8
    NTILE = QR // 16
    NT = W // _TS
    NU = B * Hkv // 2
    R = _NSLOT
    LT, TT = _LAG // 8, _TOP // 8
    scale = Dh ** -0.5
    assert W % _TS == 0 and LT < NT and 3 * TT <= NT and sum(_LAST) == N

    def kv_rows(a, t):
        sh = _SHIFT[a]
        lo, hi = t * _TS + sh, (t + 1) * _TS + sh
        rows = [(max(lo, 0), min(hi, W) - max(lo, 0))]
        if t == 0 and lo > 0:
            rows.insert(0, (0, lo))
        if t == NT - 1 and hi < W:
            rows.append((hi, W - hi))
        return rows

    sord = [4 * a + s for s in range(4) for a in range(2)]
    groups, copies = [], []

    def add_group(items, tile, c0, c1):
        for k, item in enumerate(items):
            copies.append(item + (_PAT[k % 4], len(groups)))
        groups.append((tile, c0, c1))

    for i in range(NTILE - 1):
        add_group([(st, j, c, _CC) for j in (2 * i, 2 * i + 1)
                   for c in range(0, N, _CC) for st in sord], i, 0, N)
    col = 0
    for w in _LAST:
        add_group([(st, j, c, _CC) for c in range(col, col + w, _CC)
                   for j in (NSTRIP - 2, NSTRIP - 1) for st in sord], NTILE - 1, col, col + w)
        col += w
    NG = len(groups)
    lo, hi = [], []
    for st, j, c, cc, p, g in copies:
        if p == 0 and g < NG - 1:
            hi.append((len(lo), (st, j, c, cc, 0, g)))
        else:
            lo.append((st, j, c, cc, 1, g))
    fcopies, k0 = [], 0
    for n1, item in enumerate(lo):
        while k0 < len(hi) and hi[k0][0] + _DELAY <= n1:
            fcopies.append(hi[k0][1])
            k0 += 1
        fcopies.append(item)
    fcopies.extend(item for _, item in hi[k0:])
    gend = [max(i for i, x in enumerate(fcopies) if x[5] == g) + 1 for g in range(NG)]

    def kernel(ax, ak, av, awq, awo, bx, bk, bv, bwq, bwo, out_ref,
               xbuf, wqbuf, wobuf, kvbuf, qtab, otab, zref, sem_x, sem_w, sem_k, sem_f):
        kv_arrs = (ak, av, bk, bv)
        wq_arrs = (awq, bwq)
        wo_arrs = (awo, bwo)

        zref[0] = 0

        def block(fn):
            def body(_, c):
                fn()
                return c
            lax.fori_loop(0, zref[0] + 1, body, 0)

        def unit_bh(u, j):
            return u // (Hkv // 2), u % (Hkv // 2) + (Hkv // 2) * j

        def issue_k(u, t0, t1, pinned=True):
            if t1 <= t0:
                return

            def go():
                slot = u % R
                for t in range(t0, t1):
                    for j in range(2):
                        b, h = unit_bh(u, j)
                        for a in range(4):
                            for r0, nr in kv_rows(a, t):
                                pltpu.make_async_copy(
                                    kv_arrs[a].at[b, h, pl.ds(Sk - W + r0, nr), :],
                                    kvbuf.at[slot, j * 4 + a, pl.ds(r0, nr), :],
                                    sem_k.at[slot]).start(priority=_KPAT[a])
            if pinned:
                block(go)
            else:
                go()

        def issue_rel(u, t0, t1, pinned=True):
            issue_k(u, t0, min(t1, NT), pinned)
            issue_k(u + 1, max(t0, NT) - NT, t1 - NT, pinned)

        def wait_k(u):
            slot = u % R
            pltpu.make_async_copy(kvbuf.at[slot], kvbuf.at[slot], sem_k.at[slot]).wait()

        fpos = [0]

        def issue_f(upto):
            upto = min(upto, len(fcopies))
            if upto <= fpos[0]:
                return
            items = fcopies[fpos[0]:upto]
            fpos[0] = upto

            def go():
                z = zref[0]
                for st, j, c, cc, p, g in items:
                    i = j // 2
                    dst = 16 * ((st + i) % 8) + 8 * (j % 2)
                    pltpu.make_async_copy(
                        wo_arrs[st // 4].at[pl.ds(QR * (st % 4) + 8 * j, 8), pl.ds(c, cc)],
                        wobuf.at[i, pl.ds(dst, 8), pl.ds(c, cc)],
                        sem_f.at[g + z]).start(priority=p)
            block(go)

        def wait_f(g):
            i, c0, c1 = groups[g]
            r = wobuf.at[i, :, pl.ds(c0, c1 - c0)]
            pltpu.make_async_copy(r, r, sem_f.at[g]).wait()

        row = lax.broadcasted_iota(jnp.int32, (8, Dh), 0)
        lane = lax.broadcasted_iota(jnp.int32, (8, Dh), 1)

        xcp = [pltpu.make_async_copy(x, xbuf.at[i], sem_x.at[i])
               for i, x in enumerate((ax, bx))]
        for c in xcp:
            c.start()

        def issue_w(j, carry):
            for c in range(0, N, _CC):
                for k, st in enumerate(sord):
                    r0 = pl.multiple_of(QR * (st % 4) + 8 * j, 8)
                    pltpu.make_async_copy(
                        wq_arrs[st // 4].at[pl.ds(r0, 8), pl.ds(c, _CC)],
                        wqbuf.at[st // 4, pl.ds(r0, 8), pl.ds(c, _CC)],
                        sem_w.at[0]).start(priority=_PAT[k % 4])
            return carry

        lax.fori_loop(0, NSTRIP, issue_w, 0)
        otab[...] = jnp.zeros_like(otab)
        for c in xcp:
            c.wait()
        x8 = []
        for p in range(2):
            xv = xbuf[p].astype(jnp.float32)
            x8.append(jnp.concatenate([xv, xv], axis=0).astype(jnp.bfloat16))
        issue_rel(0, 0, LT, pinned=False)
        pltpu.make_async_copy(wqbuf, wqbuf, sem_w.at[0]).wait()

        for k in range(8):
            p, cq = k // 4, k % 4
            q = jnp.dot(x8[p], wqbuf[p, :, cq * 1024:(cq + 1) * 1024],
                        preferred_element_type=jnp.float32)
            q = q.astype(jnp.bfloat16).astype(jnp.float32)
            for hh in range(4):
                qtab[p * Hkv + cq * 4 + hh] = jnp.where(
                    row < 4, q[:, (2 * hh) * Dh:(2 * hh + 1) * Dh],
                    q[:, (2 * hh + 1) * Dh:(2 * hh + 2) * Dh])
            issue_rel(0, LT + NT * k // 8, LT + NT * (k + 1) // 8)

        def attn(p, j, u):
            slot = u % R
            b, h = unit_bh(u, j)
            q = qtab[p * Hkv + h].astype(jnp.bfloat16)
            s = lax.dot_general(q, kvbuf[slot, j * 4 + 2 * p], (((1,), (1,)), ((), ())),
                                preferred_element_type=jnp.float32) * scale
            m = jnp.max(s, axis=-1, keepdims=True)
            e = jnp.exp(s - m)
            l = jnp.sum(e, axis=-1, keepdims=True)
            o = jnp.dot(e.astype(jnp.bfloat16), kvbuf[slot, j * 4 + 2 * p + 1],
                        preferred_element_type=jnp.float32) / l
            otab[p * Hkv + h] = jnp.where((row & 3) == b, o, otab[p * Hkv + h])

        cuts = [LT, LT + TT, LT + 2 * TT, LT + 3 * TT, LT + NT]

        def kv_step(u, carry):
            wait_k(u)
            for k in range(4):
                attn(k // 2, k % 2, u)
                issue_rel(u + 1, cuts[k], cuts[k + 1], pinned=False)
            return carry

        lax.fori_loop(0, NU - 2, kv_step, 0)
        wait_k(NU - 2)
        for k in range(4):
            attn(k // 2, k % 2, NU - 2)
            issue_k(NU - 1, cuts[k], min(cuts[k + 1], NT))
            issue_f((cuts[k + 1] - NT) * 8)
        wait_k(NU - 1)
        for k in range(4):
            attn(k // 2, k % 2, NU - 1)
            issue_f(fpos[0] + _TOP)

        pieces = []
        for h in range(Hkv):
            oa, ob = otab[h], otab[Hkv + h]
            pieces.append(jnp.where(row < 4, oa, pltpu.roll(ob, 4, axis=0)).astype(jnp.bfloat16))
            pieces.append(jnp.where(row < 4, pltpu.roll(oa, 4, axis=0), ob).astype(jnp.bfloat16))
        olhs = jnp.concatenate(pieces, axis=1)
        acc = None
        for g in range(NG):
            i, c0, c1 = groups[g]
            issue_f(max(gend[g] + _LAG, fpos[0] + _TOP))
            wait_f(g)
            res = lax.dot_general(olhs[:, c0:c1], wobuf[i, :, c0:c1], (((1,), (1,)), ((), ())),
                                  preferred_element_type=jnp.float32)
            if c0 > 0:
                res = res + acc
            if c1 < N:
                acc = res
            else:
                is_b = (((lane >> 4) + (8 - i % 8)) & 7) >= 4
                res = jnp.where(is_b, pltpu.roll(res, 4, axis=0), res)
                res = res[:B].astype(out_ref.dtype)
                for st in range(8):
                    l0 = 16 * ((st + i) % 8)
                    oc = QR * st + 16 * i
                    out_ref[:, oc:oc + 16] = res[:, l0:l0 + 16]

    params = dict(vmem_limit_bytes=48 * 1024 * 1024, disable_bounds_checks=True)
    if hasattr(pltpu.CompilerParams, "disable_semaphore_checks"):
        params["disable_semaphore_checks"] = True
    hbm = pl.BlockSpec(memory_space=pltpu.MemorySpace.HBM)
    out = pl.pallas_call(
        kernel,
        in_specs=[hbm] * 10,
        out_specs=pl.BlockSpec(memory_space=pltpu.VMEM),
        out_shape=jax.ShapeDtypeStruct((B, 2 * D), A_x.dtype),
        scratch_shapes=[
            pltpu.VMEM((2, B, D), jnp.bfloat16),
            pltpu.VMEM((2, D, N), jnp.bfloat16),
            pltpu.VMEM((NTILE, 128, N), jnp.bfloat16),
            pltpu.VMEM((R, 8, W, Dh), jnp.bfloat16),
            pltpu.VMEM((2 * Hkv, 8, Dh), jnp.float32),
            pltpu.VMEM((2 * Hkv, 8, Dh), jnp.float32),
            pltpu.SMEM((1,), jnp.int32),
            pltpu.SemaphoreType.DMA((2,)),
            pltpu.SemaphoreType.DMA((1,)),
            pltpu.SemaphoreType.DMA((R,)),
            pltpu.SemaphoreType.DMA((NG,)),
        ],
        compiler_params=pltpu.CompilerParams(**params),
    )(A_x.reshape(B, D), A_k_cache, A_v_cache, A_wq, A_wo.T,
      B_x.reshape(B, D), B_k_cache, B_v_cache, B_wq, B_wo.T)
    return out.reshape(B, 1, 2 * D)
```

```python
import jax
import jax.numpy as jnp
from jax import lax
import jax.experimental.pallas as pl
import jax.experimental.pallas.tpu as pltpu

_HQ = 32
_DH = 128
_TS = 128
_CC = 1024
_PAT = (0, 1, 1, 1)
_KPAT = (1, 0, 1, 1)
_LAG = 96
_TOP = 24
_LAST = (2048, 1024, 1024)
_DELAY = 16
_NSLOT = 3
_SHIFT = (0, 0, 16, 16)


@jax.jit
def pallas_concat_heads__sliding_block_cached__sliding_block_cached__decode_kernel(
    A_x: jax.Array,
    A_k_cache: jax.Array,
    A_v_cache: jax.Array,
    A_wq: jax.Array,
    A_wo: jax.Array,
    B_x: jax.Array,
    B_k_cache: jax.Array,
    B_v_cache: jax.Array,
    B_wq: jax.Array,
    B_wo: jax.Array,
):
    B, Sq, D = A_x.shape
    _, Hkv, Sk, Dh = A_k_cache.shape
    assert Sq == 1 and B == 4 and D == 576 and Dh == _DH and _HQ == 2 * Hkv
    W = min(4096, max(256, Sk // 4))
    N = _HQ * Dh
    QR = D // 4
    NSTRIP = QR // 8
    NTILE = QR // 16
    NT = W // _TS
    NU = B * Hkv // 2
    R = _NSLOT
    LT, TT = _LAG // 8, _TOP // 8
    scale = Dh ** -0.5
    assert W % _TS == 0 and LT < NT and 3 * TT <= NT and sum(_LAST) == N

    def kv_rows(a, t):
        sh = _SHIFT[a]
        lo, hi = t * _TS + sh, (t + 1) * _TS + sh
        rows = [(max(lo, 0), min(hi, W) - max(lo, 0))]
        if t == 0 and lo > 0:
            rows.insert(0, (0, lo))
        if t == NT - 1 and hi < W:
            rows.append((hi, W - hi))
        return rows

    sord = [4 * a + s for s in range(4) for a in range(2)]
    groups, copies = [], []

    def add_group(items, tile, c0, c1):
        for k, item in enumerate(items):
            copies.append(item + (_PAT[k % 4], len(groups)))
        groups.append((tile, c0, c1))

    for i in range(NTILE - 1):
        add_group([(st, j, c, _CC) for j in (2 * i, 2 * i + 1)
                   for c in range(0, N, _CC) for st in sord], i, 0, N)
    col = 0
    for w in _LAST:
        add_group([(st, j, c, _CC) for c in range(col, col + w, _CC)
                   for j in (NSTRIP - 2, NSTRIP - 1) for st in sord], NTILE - 1, col, col + w)
        col += w
    NG = len(groups)
    lo, hi = [], []
    for st, j, c, cc, p, g in copies:
        if p == 0 and g < NG - 1:
            hi.append((len(lo), (st, j, c, cc, 0, g)))
        else:
            lo.append((st, j, c, cc, 1, g))
    fcopies, k0 = [], 0
    for n1, item in enumerate(lo):
        while k0 < len(hi) and hi[k0][0] + _DELAY <= n1:
            fcopies.append(hi[k0][1])
            k0 += 1
        fcopies.append(item)
    fcopies.extend(item for _, item in hi[k0:])
    gend = [max(i for i, x in enumerate(fcopies) if x[5] == g) + 1 for g in range(NG)]

    def kernel(ax, ak, av, awq, awo, bx, bk, bv, bwq, bwo, out_ref,
               xbuf, wqbuf, wobuf, kvbuf, qtab, otab, sem_x, sem_w, sem_k, sem_f):
        kv_arrs = (ak, av, bk, bv)
        wq_arrs = (awq, bwq)
        wo_arrs = (awo, bwo)

        zero = pl.program_id(0)

        def block(fn):
            def body(_, c):
                fn()
                return c
            lax.fori_loop(0, zero + 1, body, 0)

        def unit_bh(u, j):
            return u // (Hkv // 2), u % (Hkv // 2) + (Hkv // 2) * j

        def issue_k(u, t0, t1, pinned=True):
            if t1 <= t0:
                return

            def go():
                slot = u % R
                for t in range(t0, t1):
                    for j in range(2):
                        b, h = unit_bh(u, j)
                        for a in range(4):
                            for r0, nr in kv_rows(a, t):
                                pltpu.make_async_copy(
                                    kv_arrs[a].at[b, h, pl.ds(Sk - W + r0, nr), :],
                                    kvbuf.at[slot, j * 4 + a, pl.ds(r0, nr), :],
                                    sem_k.at[slot]).start(priority=_KPAT[a])
            if pinned:
                block(go)
            else:
                go()

        def issue_rel(u, t0, t1, pinned=True):
            issue_k(u, t0, min(t1, NT), pinned)
            issue_k(u + 1, max(t0, NT) - NT, t1 - NT, pinned)

        def wait_k(u):
            slot = u % R
            pltpu.make_async_copy(kvbuf.at[slot], kvbuf.at[slot], sem_k.at[slot]).wait()

        fpos = [0]

        def issue_f(upto):
            upto = min(upto, len(fcopies))
            if upto <= fpos[0]:
                return
            items = fcopies[fpos[0]:upto]
            fpos[0] = upto

            def go():
                for st, j, c, cc, p, g in items:
                    i = j // 2
                    dst = 16 * ((st + i) % 8) + 8 * (j % 2)
                    pltpu.make_async_copy(
                        wo_arrs[st // 4].at[pl.ds(QR * (st % 4) + 8 * j, 8), pl.ds(c, cc)],
                        wobuf.at[i, pl.ds(dst, 8), pl.ds(c, cc)],
                        sem_f.at[g]).start(priority=p)
            block(go)

        def wait_f(g):
            i, c0, c1 = groups[g]
            r = wobuf.at[i, :, pl.ds(c0, c1 - c0)]
            pltpu.make_async_copy(r, r, sem_f.at[g]).wait()

        row = lax.broadcasted_iota(jnp.int32, (8, Dh), 0)
        lane = lax.broadcasted_iota(jnp.int32, (8, Dh), 1)

        xcp = [pltpu.make_async_copy(x, xbuf.at[i], sem_x.at[i])
               for i, x in enumerate((ax, bx))]
        for c in xcp:
            c.start()

        def issue_w(j, carry):
            for c in range(0, N, _CC):
                for k, st in enumerate(sord):
                    r0 = pl.multiple_of(QR * (st % 4) + 8 * j, 8)
                    pltpu.make_async_copy(
                        wq_arrs[st // 4].at[pl.ds(r0, 8), pl.ds(c, _CC)],
                        wqbuf.at[st // 4, pl.ds(r0, 8), pl.ds(c, _CC)],
                        sem_w.at[0]).start(priority=_PAT[k % 4])
            return carry

        lax.fori_loop(0, NSTRIP, issue_w, 0)
        otab[...] = jnp.zeros_like(otab)
        for c in xcp:
            c.wait()
        x8 = []
        for p in range(2):
            xv = xbuf[p].astype(jnp.float32)
            x8.append(jnp.concatenate([xv, xv], axis=0).astype(jnp.bfloat16))
        issue_rel(0, 0, LT, pinned=False)
        pltpu.make_async_copy(wqbuf, wqbuf, sem_w.at[0]).wait()

        for k in range(8):
            p, cq = k // 4, k % 4
            q = jnp.dot(x8[p], wqbuf[p, :, cq * 1024:(cq + 1) * 1024],
                        preferred_element_type=jnp.float32)
            q = q.astype(jnp.bfloat16).astype(jnp.float32)
            for hh in range(4):
                qtab[p * Hkv + cq * 4 + hh] = jnp.where(
                    row < 4, q[:, (2 * hh) * Dh:(2 * hh + 1) * Dh],
                    q[:, (2 * hh + 1) * Dh:(2 * hh + 2) * Dh])
            issue_rel(0, LT + NT * k // 8, LT + NT * (k + 1) // 8)

        def attn(p, j, u):
            slot = u % R
            b, h = unit_bh(u, j)
            q = qtab[p * Hkv + h].astype(jnp.bfloat16)
            s = lax.dot_general(q, kvbuf[slot, j * 4 + 2 * p], (((1,), (1,)), ((), ())),
                                preferred_element_type=jnp.float32) * scale
            m = jnp.max(s, axis=-1, keepdims=True)
            e = jnp.exp(s - m)
            l = jnp.sum(e, axis=-1, keepdims=True)
            o = jnp.dot(e.astype(jnp.bfloat16), kvbuf[slot, j * 4 + 2 * p + 1],
                        preferred_element_type=jnp.float32) / l
            otab[p * Hkv + h] = jnp.where((row & 3) == b, o, otab[p * Hkv + h])

        cuts = [LT, LT + TT, LT + 2 * TT, LT + 3 * TT, LT + NT]

        def kv_step(u, carry):
            wait_k(u)
            for k in range(4):
                attn(k // 2, k % 2, u)
                issue_rel(u + 1, cuts[k], cuts[k + 1], pinned=False)
            return carry

        lax.fori_loop(0, NU - 2, kv_step, 0)
        wait_k(NU - 2)
        for k in range(4):
            attn(k // 2, k % 2, NU - 2)
            issue_k(NU - 1, cuts[k], min(cuts[k + 1], NT))
            issue_f((cuts[k + 1] - NT) * 8)
        wait_k(NU - 1)
        for k in range(4):
            attn(k // 2, k % 2, NU - 1)
            issue_f(fpos[0] + _TOP)

        pieces = []
        for h in range(Hkv):
            oa, ob = otab[h], otab[Hkv + h]
            pieces.append(jnp.where(row < 4, oa, pltpu.roll(ob, 4, axis=0)).astype(jnp.bfloat16))
            pieces.append(jnp.where(row < 4, pltpu.roll(oa, 4, axis=0), ob).astype(jnp.bfloat16))
        olhs = jnp.concatenate(pieces, axis=1)
        acc = None
        for g in range(NG):
            i, c0, c1 = groups[g]
            issue_f(max(gend[g] + _LAG, fpos[0] + _TOP))
            wait_f(g)
            res = lax.dot_general(olhs[:, c0:c1], wobuf[i, :, c0:c1], (((1,), (1,)), ((), ())),
                                  preferred_element_type=jnp.float32)
            if c0 > 0:
                res = res + acc
            if c1 < N:
                acc = res
            else:
                is_b = (((lane >> 4) + (8 - i % 8)) & 7) >= 4
                res = jnp.where(is_b, pltpu.roll(res, 4, axis=0), res)
                res = res[:B].astype(out_ref.dtype)
                for st in range(8):
                    l0 = 16 * ((st + i) % 8)
                    oc = QR * st + 16 * i
                    out_ref[:, oc:oc + 16] = res[:, l0:l0 + 16]

    params = dict(vmem_limit_bytes=48 * 1024 * 1024, disable_bounds_checks=True)
    if hasattr(pltpu.CompilerParams, "disable_semaphore_checks"):
        params["disable_semaphore_checks"] = True
    hbm = pl.BlockSpec(memory_space=pltpu.MemorySpace.HBM)
    out = pl.pallas_call(
        kernel,
        grid=(1,),
        in_specs=[hbm] * 10,
        out_specs=pl.BlockSpec((B, 2 * D), lambda i: (0, 0)),
        out_shape=jax.ShapeDtypeStruct((B, 2 * D), A_x.dtype),
        scratch_shapes=[
            pltpu.VMEM((2, B, D), jnp.bfloat16),
            pltpu.VMEM((2, D, N), jnp.bfloat16),
            pltpu.VMEM((NTILE, 128, N), jnp.bfloat16),
            pltpu.VMEM((R, 8, W, Dh), jnp.bfloat16),
            pltpu.VMEM((2 * Hkv, 8, Dh), jnp.float32),
            pltpu.VMEM((2 * Hkv, 8, Dh), jnp.float32),
            pltpu.SemaphoreType.DMA((2,)),
            pltpu.SemaphoreType.DMA((1,)),
            pltpu.SemaphoreType.DMA((R,)),
            pltpu.SemaphoreType.DMA((NG,)),
        ],
        compiler_params=pltpu.CompilerParams(**params),
    )(A_x.reshape(B, D), A_k_cache, A_v_cache, A_wq, A_wo.T,
      B_x.reshape(B, D), B_k_cache, B_v_cache, B_wq, B_wo.T)
    return out.reshape(B, 1, 2 * D)
```
